```python
import os as _os
_os.environ.setdefault("JAX_PLATFORMS", "cpu")
import jax
import jax.numpy as jnp

def _softmax(x, axis=-1):
    return jax.nn.softmax(x, axis=axis)
def _gelu(x):
    return jax.nn.gelu(x, approximate=True)
def _silu(x):
    return jax.nn.silu(x)
def _sigmoid(x):
    return jax.nn.sigmoid(x)
def _layernorm(x, axis=-1, eps=1e-5):
    m = jnp.mean(x, axis=axis, keepdims=True)
    v = jnp.var(x, axis=axis, keepdims=True)
    return (x - m) / jnp.sqrt(v + eps)
def _scatter_add(tgt, idx, src, axis=0):
    return tgt.at[idx].add(src)
def _segment_sum(src, seg, n):
    return jax.ops.segment_sum(src, seg, n)
class _Rng:
    def __init__(self, key):
        self._k = key
    def _next(self):
        self._k, sub = jax.random.split(self._k)
        return sub
    def normal(self, shape):
        return jax.random.normal(self._next(), shape, dtype=jnp.bfloat16)
    def randint(self, lo, hi, shape):
        return jax.random.randint(self._next(), shape, lo, hi, dtype=jnp.int32)
    def uniform(self, shape, lo=0.0, hi=1.0):
        return jax.random.uniform(self._next(), shape, jnp.bfloat16, lo, hi)
    def permutation(self, n):
        return jax.random.permutation(self._next(), n)


kernel_name = 'standalone__layernorm_linear__sampling'

def setup_inputs():
    _rng = _Rng(jax.random.key(int.from_bytes(__import__("os").urandom(4), "little")))
    _w = (lambda a: (lambda t: t.astype(jnp.bfloat16) if jnp.issubdtype(t.dtype, jnp.floating) else t)(jnp.asarray(a)))
    B, S, D = 1024, 32, 576
    return {
        "x": _w((lambda *s: _rng.normal(s) * 0.05)(B, S, D)),
        "g": _w((lambda *s: _rng.normal(s) * 0.05)(D) + 1.0),
        "b": _w((lambda *s: _rng.normal(s) * 0.05)(D)),
        "w": _w((lambda *s: _rng.normal(s) * 0.05)(D, D)),
    }

def reference(x, g, b, w):
    return (_layernorm(x, axis=-1) * g + b) @ w
```

```python
import functools
import jax, jax.numpy as jnp
from jax import lax
import jax.experimental.pallas as pl
import jax.experimental.pallas.tpu as pltpu

F32 = jnp.float32
BF16 = jnp.bfloat16
U32 = jnp.uint32
KH = 256
K3 = 80
TW = 128
EPS = 1e-5

pk = lambda t: pltpu.bitcast(t.astype(BF16), U32)
up = lambda t: pltpu.bitcast(t, BF16)
bits = lambda t: pltpu.bitcast(t, U32)
flt = lambda t: pltpu.bitcast(t, F32)

def dot(a, b):
    return jnp.dot(a, b, preferred_element_type=F32)

def prep_weights(g_ref, b_ref, w_ref, a_ref, a3_ref, D):
    H = D // 2
    w = w_ref[...]
    g = g_ref[...].astype(F32).reshape(1, D)
    b16 = jnp.broadcast_to(b_ref[...].reshape(1, D), (16, D))
    bias = dot(b16, w)[0:1]
    b_hi = bias.astype(BF16).astype(F32)
    r1 = bias - b_hi
    b_mid = r1.astype(BF16).astype(F32)
    b_lo = r1 - b_mid
    row = lax.broadcasted_iota(jnp.int32, (64, D), 0)
    ext = jnp.where(row == 0, b_hi, jnp.where(row == 1, b_mid, jnp.where(row == 2, b_lo, 0.0)))
    T = lambda blk: blk.T.astype(F32)
    cols = [T(w[kt*128:(kt+1)*128, :]) * g[:, kt*128:(kt+1)*128] for kt in range(4)]
    last = jnp.concatenate([w[2*KH:, :], ext.astype(BF16)], axis=0)
    g3 = jnp.concatenate([g[:, 2*KH:], jnp.ones((1, 64), F32)], axis=1)
    a3_ref[...] = pk(T(last) * g3)
    L = jnp.concatenate(cols[:2], axis=1); Rr = jnp.concatenate(cols[2:], axis=1)
    A11 = L[:H]; A21 = L[H:]; A12 = Rr[:H]; A22 = Rr[H:]
    ops = [A11 + A22, A21 + A22, A11, A22, A11 + A12, A21 - A11, A12 - A22]
    for i, a in enumerate(ops):
        a_ref[i * (H // 2):(i + 1) * (H // 2), :] = pk(a)


def build(head=((256,), (256,), (512,), (1024,), (1024, 1024)), nloop=4,
          tail=(1024, 1024, 1024, 512, 256, 256), iw=2, nodma=0):
    def kern(x_hbm, g_hbm, b_hbm, w_hbm, o_hbm, xbuf, obuf, g_ref, b_ref, w_ref, a_ref, a3_ref, st_ref, sem_all, wsem):
        psem = sem_all; rsem = sem_all.at[pl.ds(3, sem_all.shape[0] - 3)]
        S, D, B = x_hbm.shape
        H = D // 2
        pos = 0
        def take(widths):
            nonlocal pos
            out = []
            for w_ in widths:
                assert pos % B + w_ <= B
                out.append((pos // B, pos % B, w_)); pos += w_
            return out
        head_regions = [take(r) for r in head]
        assert pos % B == 0
        s_loop = pos // B
        tail_cols = sum(tail)
        assert tail_cols % B == 0
        s_tail = S - tail_cols // B
        assert (s_tail - s_loop) % nloop == 0
        NG = (s_tail - s_loop) // nloop
        pos = s_tail * B
        tail_region = take(tail)
        assert tail_region[0][2] == B or NG == 0

        def rd_chunk(ch, k):
            s, c0, w_ = ch
            return pltpu.make_async_copy(x_hbm.at[s, :, pl.ds(c0, w_)], xbuf.at[s, :, pl.ds(c0, w_)], rsem.at[k])
        def rd_slabs(s, m, k):
            return pltpu.make_async_copy(x_hbm.at[pl.ds(s, m)], xbuf.at[pl.ds(s, m)], rsem.at[k])
        class _Nop:
            def start(self): pass
            def wait(self): pass
        if nodma & 1:
            rd_chunk = lambda ch, k: _Nop()
            rd_slabs = lambda s, m, k: _Nop()
        def wr(s, r0, nr, c0, w_):
            if nodma & 2 and nr == D: return
            pltpu.make_async_copy(obuf.at[s, pl.ds(r0, nr), pl.ds(c0, w_)], o_hbm.at[s, pl.ds(r0, nr), pl.ds(c0, w_)], wsem.at[0]).start()

        def wr_slabs(s, m):
            if nodma & 2: return
            pltpu.make_async_copy(obuf.at[pl.ds(s, m)], o_hbm.at[pl.ds(s, m)], wsem.at[0]).start()
        params = [pltpu.make_async_copy(w_hbm, w_ref, psem.at[0]),
                  pltpu.make_async_copy(g_hbm, g_ref, psem.at[1]),
                  pltpu.make_async_copy(b_hbm, b_ref, psem.at[2])]
        for p in params: p.start()
        head_chunks = [c for r in head_regions for c in r]
        head_rd = [rd_chunk(c, k) for k, c in enumerate(head_chunks)]
        nh = len(head_chunks)
        for cp in head_rd: cp.start()
        first_rd = rd_slabs(s_loop, 1, nh)
        first_rd.start()
        for i in range(NG): rd_slabs(s_loop + 1 + i * nloop, nloop, nh + 1 + i).start()
        rest = S - s_tail - 1
        if NG == 0: rest = S - s_loop - 1
        tail_rd = rd_slabs(S - rest, rest, nh + 1 + NG) if rest else None
        if tail_rd is not None: tail_rd.start()

        for p in params: p.wait()
        prep_weights(g_ref, b_ref, w_ref, a_ref, a3_ref, D)

        def stats_tile(s, c0):
            ld = lambda r: xbuf[s, r:r + 8, c0:c0 + TW].astype(F32)
            first = ld(0)
            cc = jnp.broadcast_to(first[0:1, :], (8, TW))
            d = first - cc
            a1 = d; a2 = d * d
            for r in range(8, D, 8):
                d = ld(r) - cc
                a1 = a1 + d
                a2 = a2 + d * d
            s1 = jnp.sum(a1, axis=0, keepdims=True) * (1.0 / D)
            s2 = jnp.sum(a2, axis=0, keepdims=True) * (1.0 / D)
            m = cc[0:1, :] + s1
            v = jnp.maximum(s2 - s1 * s1, 0.0)
            return m, lax.rsqrt(v + EPS)

        def cat(ts): return ts[0] if len(ts) == 1 else jnp.concatenate(ts, axis=1)

        def chunk(ch, stat, nxt, write=True, fine=False):
            s, c0, cn = ch
            h = cn // 2
            m, rr = stat
            nt = nxt[2] // TW if nxt is not None else 0
            plan = [0] * 9
            for t in range(nt): plan[1 + (t * 8) // nt] += 1
            ms, rs = [], []
            cnt = [0]
            def post(r):
                for _ in range(plan[cnt[0]]):
                    m_, r_ = stats_tile(nxt[0], nxt[1] + len(ms) * TW)
                    ms.append(m_); rs.append(r_)
                    tok = jnp.broadcast_to(bits(r_) >> 31, (8, TW))
                    k0 = ((len(ms) - 1) % (r.shape[1] // TW)) * TW
                    blk = flt(bits(r[0:8, k0:k0 + TW]) | tok)
                    row = cat(([r[0:8, :k0]] if k0 else []) + [blk] + ([r[0:8, k0 + TW:]] if k0 + TW < r.shape[1] else []))
                    r = jnp.concatenate([row, r[8:]], axis=0)
                cnt[0] += 1
                return r
            bf = lambda t: t.astype(BF16)
            xn = (xbuf[s, :, c0:c0 + cn].astype(F32) - m) * rr
            B11 = xn[:KH, :h]; B12 = xn[:KH, h:]; B21 = xn[KH:2*KH, :h]; B22 = xn[KH:2*KH, h:]
            Bop = [lambda: B11 + B22, lambda: B11, lambda: B12 - B22, lambda: B21 - B11, lambda: B22, lambda: B11 + B12, lambda: B21 + B22]
            A = lambda i: up(a_ref[i * (H // 2):(i + 1) * (H // 2), :])
            M = lambda i: post(dot(A(i - 1), bf(Bop[i - 1]())))
            def out(r0, k0, v): obuf[s, r0:r0 + H, c0 + k0:c0 + k0 + h] = v.astype(BF16)
            b3 = jnp.concatenate([bf(xn[2*KH:, :]), jnp.ones((K3 - 64, cn), BF16)], axis=0)
            Rb = post(dot(up(a3_ref[H // 2:, :])[:, :K3], b3))
            M2 = M(2); P21 = Rb[:, :h] + M2; P22 = Rb[:, h:] - M2
            M4 = M(4); out(H, 0, P21 + M4)
            M1 = M(1); P11 = M4 + M1; P22 = P22 + M1
            M6 = M(6); P22 = P22 + M6
            M3 = M(3); out(H, h, P22 + M3)
            if write and fine: wr(s, H, H, c0, cn)
            M5 = M(5); P11 = P11 - M5; P12 = M3 + M5
            M7 = M(7); P11 = P11 + M7
            Rt = post(dot(up(a3_ref[:H // 2, :])[:, :K3], b3))
            out(0, 0, P11 + Rt[:, :h]); out(0, h, P12 + Rt[:, h:])
            if write:
                if fine: wr(s, 0, H, c0, cn)
                else: wr(s, 0, D, c0, cn)
            return (cat(ms), cat(rs)) if nt else None

        head_rd[0].wait()
        c = head_chunks[0]
        tiles = [stats_tile(c[0], c[1] + t * TW) for t in range(c[2] // TW)]
        stat = (cat([t[0] for t in tiles]), cat([t[1] for t in tiles]))
        k = 0
        after_head = (s_loop, 0, B) if NG else tail_region[0]
        pending = []
        for ri, reg in enumerate(head_regions):
            for j in range(len(reg)):
                if k + j + 1 < nh: head_rd[k + j + 1].wait()
                else: first_rd.wait()
            for j, ch in enumerate(reg):
                nxt = head_chunks[k + j + 1] if k + j + 1 < nh else after_head
                stat = chunk(ch, stat, nxt, write=False)
            k += len(reg)

        if NG:
            st_ref[0:1, :] = stat[0]; st_ref[1:2, :] = stat[1]
            def body(i, carry):
                s0 = s_loop + i * nloop
                @pl.when(i == iw)
                def _(): wr_slabs(0, s_loop + iw * nloop)
                @pl.when(i > iw)
                def _(): wr_slabs(s0 - nloop, nloop)
                rd_slabs(s0 + 1, nloop, nh + 1 + i).wait()
                stat = (st_ref[0:1, :], st_ref[1:2, :])
                for j in range(nloop):
                    stat = chunk((s0 + j, 0, B), stat, (s0 + j + 1, 0, B), write=False)
                st_ref[0:1, :] = stat[0]; st_ref[1:2, :] = stat[1]
                return carry
            lax.fori_loop(0, NG, body, 0)
            stat = (st_ref[0:1, :], st_ref[1:2, :])
            assert iw < NG
            wr_slabs(s_tail - nloop, nloop)

        if tail_rd is not None: tail_rd.wait()
        for j, ch in enumerate(tail_region):
            nxt = tail_region[j + 1] if j + 1 < len(tail_region) else None
            stat = chunk(ch, stat, nxt, fine=(nxt is None))
        if nodma & 2:
            s, c0, cn = tail_region[-1]
            pltpu.make_async_copy(obuf.at[s, :, pl.ds(c0, cn)], o_hbm.at[s, :, pl.ds(c0, cn)], wsem.at[0]).wait()
        else:
            pltpu.make_async_copy(obuf, o_hbm, wsem.at[0]).wait()

    @jax.jit
    def f(x, g, b, w):
        B, S, D = x.shape
        xt = jnp.transpose(x, (1, 2, 0))
        nsem = sum(len(r) for r in head) + 2 + S
        nsem = sum(len(r) for r in head) + 2 + (S - sum(sum(r) for r in head) // B - sum(tail) // B) // nloop
        out = pl.pallas_call(
            kern,
            in_specs=[pl.BlockSpec(memory_space=pl.ANY)] * 4,
            out_specs=pl.BlockSpec(memory_space=pl.ANY),
            out_shape=jax.ShapeDtypeStruct((S, D, B), x.dtype),
            scratch_shapes=[
                pltpu.VMEM((S, D, B), BF16), pltpu.VMEM((S, D, B), BF16),
                pltpu.VMEM((D,), BF16), pltpu.VMEM((D,), BF16), pltpu.VMEM((D, D), BF16),
                pltpu.VMEM((7 * D // 4, KH), U32), pltpu.VMEM((D // 2, 128), U32),
                pltpu.VMEM((8, B), F32),
                pltpu.SemaphoreType.DMA((3 + nsem,)), pltpu.SemaphoreType.DMA((1,)),
            ],
            compiler_params=pltpu.CompilerParams(vmem_limit_bytes=110*1024*1024),
        )(xt, g, b, w)
        return jnp.transpose(out, (2, 0, 1))
    return f


_impl = build()


@jax.jit
def pallas_standalone__layernorm_linear__sampling_kernel(x, g, b, w):
    return _impl(x, g, b, w)
```

```python
import functools

import jax
import jax.numpy as jnp
from jax import lax
import jax.experimental.pallas as pl
import jax.experimental.pallas.tpu as pltpu

F32 = jnp.float32
BF16 = jnp.bfloat16
U32 = jnp.uint32
KH = 256
K3 = 80
TW = 128
EPS = 1e-5
QUADS = ((0, 0), (0, 1), (1, 0), (1, 1))
CN = 512

pk = lambda t: pltpu.bitcast(t.astype(BF16), U32)
up = lambda t: pltpu.bitcast(t, BF16)
bits = lambda t: pltpu.bitcast(t, U32)
flt = lambda t: pltpu.bitcast(t, F32)
bf = lambda t: t.astype(BF16)


def dot(a, b):
    return jnp.dot(a, b, preferred_element_type=F32)


def cat(ts, axis=1):
    return ts[0] if len(ts) == 1 else jnp.concatenate(ts, axis=axis)


def quads(t):
    r, c = t.shape[0] // 2, t.shape[1] // 2
    return t[:r, :c], t[:r, c:], t[r:, :c], t[r:, c:]


def lhs_op(k, a11, a12, a21, a22):
    return {1: lambda: a11 - a22, 2: lambda: a21 - a22, 3: lambda: a11, 4: lambda: a22,
            5: lambda: a12 - a11, 6: lambda: a11 - a21, 7: lambda: a12 - a22}[k]()


def rhs_op(k, b11, b12, b21, b22):
    return {1: lambda: b11 + b22, 2: lambda: b11, 3: lambda: b12 + b22, 4: lambda: b21 + b11,
            5: lambda: b22, 6: lambda: b11 - b12, 7: lambda: b21 - b22}[k]()


USERS = {1: (((0, 0), 1), ((1, 1), -1)), 2: (((1, 0), 1), ((1, 1), 1)), 3: (((0, 1), 1), ((1, 1), 1)),
         4: (((0, 0), 1), ((1, 0), 1)), 5: (((0, 0), 1), ((0, 1), 1)), 6: (((1, 1), 1),), 7: (((0, 0), 1),)}
NTERMS = {(0, 0): 5, (0, 1): 3, (1, 0): 3, (1, 1): 5}
RHS_USES = {1: (0, 3), 2: (0,), 3: (1, 3), 4: (2, 0), 5: (3,), 6: (0, 1), 7: (2, 3)}

CFG = {
    ('H', 0): ('2b6517t43', '6413725 5241637 6214375 2473156 2653417 4712653 2475361', '000100111', '103560033'),
    ('H', 1): ('2b4t65713', '5624137 5241637 2641375 2457163 2653417 4751263 3472561', '001011001', '326330030'),
    ('H', 2): ('2b4t65713', '6241735 5271634 2641375 2415736 2653417 4751263 2475361', '001001101', '143430330'),
    ('H', 3): ('2b4t65713', '1624357 5241637 2641375 2451736 6145327 4752361 2475361', '000210001', '103530030'),
    ('H', 4): ('2b4t65713', '6142735 5241637 2461375 2451736 2563417 4751263 2471536', '001101001', '503530630'),
    ('H', 5): ('2b4t65713', '5143762 2514637 2146735 2415736 2643517 4751263 2475361', '001101001', '103530030'),
    ('H', 6): ('2b4t65713', '6241357 5214637 4263175 2174536 2653417 4751263 3427615', '001101001', '104632031'),
    ('L', 0): ('t24b65713', '6241357 5241376 2641357 2415736 2654317 4752163 2673451', '001101001', '022100210'),
    ('L', 1): ('2b4t65713', '6241357 3564271 2641357 2415736 2645317 4752163 4372651', '001101001', '243100310'),
    ('L', 2): ('2b4t65713', '6274351 5241376 2641357 2415736 2654317 4752361 2473651', '001101001', '352100310'),
    ('L', 3): ('2b4t65713', '6241357 5241673 2641357 2415736 2654317 4752163 4736512', '001101001', '242000310'),
    ('L', 4): ('2b4t65713', '6241357 5241376 2614357 2415736 2654317 4752163 2673451', '001101001', '242600310'),
    ('L', 5): ('2b4t65713', '7241356 3524671 2641357 2415736 2645317 4751263 4372651', '000201001', '243100310'),
    ('L', 6): ('2b4t65713', '6143572 5241376 2764135 2415736 2654317 5742361 2473651', '001101001', '352100310'),
    ('L', 7): ('2b4t65713', '6241375 5241376 2641357 2415736 2654317 4752163 2473651', '001101001', '241000313'),
    ('P', 0): ('t24b65713', '6241357 5324176 2641357 2415736 2654317 4752163 2473651', '001101001', '022100310'),
    ('P', 1): ('2b4t65713', '6241357 3564271 2641357 2315746 2654317 4752163 4732651', '001101001', '243100310'),
    ('P', 2): ('2b4t65713', '6214357 5241376 2641357 2415736 2654317 4752361 2473651', '001101001', '254100310'),
    ('P', 3): ('2b4t65713', '6241357 5241673 2641375 2415736 2654317 4752163 4736512', '001101001', '242000310'),
    ('P', 4): ('2b4t65713', '6241357 5241376 2614357 3415726 2654317 4752163 2473651', '001101001', '242100310'),
    ('P', 5): ('2b4t65713', '7241356 3524671 1642357 2415736 2654317 4751263 4732651', '000201001', '243100310'),
    ('P', 6): ('2b4t65713', '6143527 5241376 2764135 2415736 2654317 5742361 2473651', '001101001', '552100310'),
    ('P', 7): ('2b4t65713', '6213475 5241376 2641357 2415736 2654317 4752163 2473651', '001101001', '242001310'),
    ('P', 8): ('2b4t63157', '6241357 5241637 2641357 2415736 2154367 4752163 2473615', '000000000', '000000000'),
}

NHEAD = 7
NLOOP = 8
NPOST = 9
IW = 3
RW = 24
DRAIN = 3
WSPLIT = 256
BARS = ((0, 2), (1, 1), (3, 0))
NSEM = 15


def build():
    def conf_of(key):
        order, subs, plan, tsub = CFG[key]
        return order, dict(enumerate(subs.split(), 1)), tuple(map(int, plan)), tuple(map(int, tsub))

    def kern(x_hbm, g_hbm, b_hbm, w_hbm, o_hbm, xbuf, obuf, g_ref, b_ref, w_ref, wt_ref, s_ref, st_ref, sem, wsem):
        S, D, B = x_hbm.shape
        H = D // 2
        Q = H // 2
        assert B == 2 * CN
        NQ = 2 * S
        nhead = NHEAD
        NG = (NQ - nhead - NPOST) // NLOOP
        SL = NLOOP // 2
        s_loop = nhead // 2
        s_post = s_loop + NG * SL
        assert nhead % 2 == 1 and nhead + NG * NLOOP + NPOST == NQ and SL % 2 == 0 and s_loop % 2 == 1
        at = lambda s0, j: (s0 + j // 2, (j % 2) * CN)

        nsem = [0]

        def new_sem():
            nsem[0] += 1
            return nsem[0] - 1

        def rd_desc(s, m, c0, w_, k):
            return pltpu.make_async_copy(x_hbm.at[pl.ds(s, m), :, pl.ds(c0, w_)],
                                         xbuf.at[pl.ds(s, m), :, pl.ds(c0, w_)], sem.at[k])

        def rd_start(s, m, c0=0, w_=B):
            d_ = rd_desc(s, m, c0, w_, new_sem())
            d_.start()
            return d_

        pend = []

        def wr_slabs(s, m, cond=None, c0=0, w_=B, rows=RW):
            for r0 in range(0, H, rows):
                def go(r0=r0):
                    pltpu.make_async_copy(obuf.at[pl.ds(2 * s, 2 * m), pl.ds(r0, rows), pl.ds(c0, w_)],
                                          o_hbm.at[pl.ds(2 * s, 2 * m), pl.ds(r0, rows), pl.ds(c0, w_)],
                                          wsem.at[0]).start()
                pend.append(go if cond is None else functools.partial(pl.when(cond), go))

        w_rd = [pltpu.make_async_copy(w_hbm.at[pl.ds(r0, n)], w_ref.at[pl.ds(r0, n)], sem.at[new_sem()])
                for r0, n in ((0, WSPLIT), (WSPLIT, D - WSPLIT))]
        gb_rd = [pltpu.make_async_copy(g_hbm, g_ref, sem.at[new_sem()]),
                 pltpu.make_async_copy(b_hbm, b_ref, sem.at[new_sem()])]
        for d_ in gb_rd + w_rd:
            d_.start()
        head_rd = [rd_start(0, 1, 0, CN), rd_start(0, 1, CN, CN), rd_start(1, 1), rd_start(2, 2)]
        assert nhead == 7
        loop_sem0 = nsem[0]
        for i in range(NG):
            rd_start(s_loop + 1 + i * SL, SL)
        post_rd = rd_start(s_post + 1, S - s_post - 1)
        assert nsem[0] <= sem.shape[0], nsem

        def stats_tile(s, c0):
            ld = lambda r: xbuf[s, pl.ds(r, 8), c0:c0 + TW].astype(F32)
            first = ld(0)
            cc = first[0:1, :]
            cb = jnp.broadcast_to(cc, (8, TW))
            d = first - cb

            def step(r, c):
                d = ld(pl.multiple_of(r * 8, 8)) - cb
                return c[0] + d, c[1] + d * d

            a1, a2 = lax.fori_loop(1, D // 8, step, (d, d * d), unroll=True)
            s1 = jnp.sum(a1, axis=0, keepdims=True) * (1.0 / D)
            s2 = jnp.sum(a2, axis=0, keepdims=True) * (1.0 / D)
            v = jnp.maximum(s2 - s1 * s1, 0.0)
            return cc + s1, lax.rsqrt(v + EPS)

        tiles_of = lambda c: [(c[0], c[1] + j * TW) for j in range(CN // TW)]

        for d_ in gb_rd + w_rd[:1]:
            d_.wait()
        g = g_ref[...].astype(F32).reshape(1, D)
        bb = b_ref[...].astype(F32).reshape(1, D)
        bg = bf(jnp.where(lax.broadcasted_iota(jnp.int32, (16, D), 0) == 0, bb, g))
        eye = (lax.broadcasted_iota(jnp.int32, (128, 128), 0)
               == lax.broadcasted_iota(jnp.int32, (128, 128), 1)).astype(BF16)

        def tr(kt):
            blk = w_ref[kt * 128:(kt + 1) * 128, :]
            if kt % 2 == 0:
                t = jnp.concatenate(
                    [lax.dot_general(eye[:min(128, D - n0), :min(128, D - n0)], blk[:, n0:min(n0 + 128, D)],
                                     (((1,), (1,)), ((), ())), preferred_element_type=F32)
                     for n0 in range(0, D, 128)], axis=0)
            else:
                t = blk.T.astype(F32)
            return t * g[:, kt * 128:(kt + 1) * 128]

        for kt in range(WSPLIT // 128):
            wt_ref[:, kt * 128:(kt + 1) * 128] = tr(kt)
        st_ref[0:16, 0:D] = dot(bg[:, :WSPLIT], w_ref[0:WSPLIT, :])
        w_rd[1].wait()
        red = st_ref[0:16, 0:D] + dot(bg[:, WSPLIT:], w_ref[WSPLIT:, :])
        for kt in range(WSPLIT // 128, 4):
            wt_ref[:, kt * 128:(kt + 1) * 128] = tr(kt)
        bias = red[0:1]
        b_hi = bias.astype(BF16).astype(F32)
        b_mid = (bias - b_hi).astype(BF16).astype(F32)
        b_lo = bias - b_hi - b_mid
        row = lax.broadcasted_iota(jnp.int32, (64, D), 0)
        ext = jnp.where(row == 0, b_hi, jnp.where(row == 1, b_mid, jnp.where(row == 2, b_lo, 0.0)))
        cen = jnp.sum(dot(bg[:, :128], w_ref[0:128, 0:128])[1:2], axis=1, keepdims=True) * (1.0 / (128 * 128))
        lastT = jnp.concatenate([w_ref[2 * KH:, :], bf(ext)], axis=0).T.astype(F32)
        lane = lax.broadcasted_iota(jnp.int32, (1, 128), 1)
        g3 = jnp.concatenate([g[:, 2 * KH:], jnp.ones((1, 64), F32)], axis=1)
        s_ref[0:H, :] = pk(lastT * g3 - jnp.where(lane < 64, cen, 0.0))
        cb16 = jnp.broadcast_to(cen, (16, 128))
        for u in range(0, Q, 16):
            V = [[wt_ref[a_ * Q + u:a_ * Q + u + 16, b_ * 128:(b_ + 1) * 128] for b_ in range(4)] for a_ in range(4)]
            for i in range(1, 8):
                Ai = [lhs_op(i, V[sa][sb], V[sa][2 + sb], V[2 + sa][sb], V[2 + sa][2 + sb]) for sa, sb in QUADS]
                for k in range(1, 8):
                    r0 = H + ((i - 1) * 7 + k - 1) * (Q // 2) + u // 2
                    v = lhs_op(k, *Ai)
                    s_ref[r0:r0 + 8, :] = pk(v - cb16 if i in (3, 4) and k in (3, 4) else v)

        def Asub(i, k):
            r0 = H + ((i - 1) * 7 + k - 1) * (Q // 2)
            return up(s_ref[r0:r0 + Q // 2, :])

        A3 = lambda half: up(s_ref[half * Q:(half + 1) * Q, :])[:, :K3]

        def chunk(ch, stat, todo, conf, mode=None, waits=None, even=()):
            s, c0 = ch
            cn = CN
            h = cn // 2
            order, subs, plan, tsub = conf
            assert sum(plan) == len(todo) and not (waits and any(plan[:max(waits) + 1]))
            m, rr = stat
            even = dict(even)
            assert all(order[p_] not in 'tb' for p_ in even)
            done, cnt = [], [0]

            def pre(r):
                nk = plan[cnt[0]]
                for kk in range(nk):
                    st = stats_tile(*todo[len(done)])
                    done.append(st)
                    tok = jnp.broadcast_to(bits(st[1]) >> 31, (8, TW))
                    k0 = ((kk * (r.shape[1] // TW)) // nk) * TW
                    blk_ = flt(bits(r[0:8, k0:k0 + TW]) | tok)
                    top = cat(([r[0:8, :k0]] if k0 else []) + [blk_]
                              + ([r[0:8, k0 + TW:]] if k0 + TW < r.shape[1] else []))
                    r = jnp.concatenate([top, r[8:]], axis=0)
                cnt[0] += 1
                for _ in range(DRAIN):
                    if pend:
                        pend.pop(0)()
                return r

            def norm(r0, r1, k):
                x = xbuf[s, r0:r1, c0 + k * h:c0 + (k + 1) * h].astype(F32)
                return (x - m[:, k * h:(k + 1) * h]) * rr[:, k * h:(k + 1) * h]

            ones = jnp.ones((K3 - 64, cn), F32)
            memo = {}

            def blk(k):
                if k not in memo:
                    memo[k] = (cat([norm(2 * KH, D, 0), norm(2 * KH, D, 1)]) if k == 4
                               else norm((k // 2) * KH, (k // 2 + 1) * KH, k % 2))
                return memo[k]

            if not waits:
                for k in range(5):
                    blk(k)
            acc = {}
            left = dict(NTERMS)

            def accum(a, key, v, sg):
                if key not in a:
                    a[key] = (v, sg)
                else:
                    u, su = a[key]
                    a[key] = (u + v, sg) if su == sg else ((u - v, 1) if su > 0 else (v - u, 1))

            def write(region):
                pltpu.make_async_copy(obuf.at[region], o_hbm.at[region], wsem.at[0]).start()

            for pos_, c in enumerate(order):
                for fn in (waits or {}).get(pos_, ()):
                    fn()
                if c in 'tb':
                    half = 'tb'.index(c)
                    r = dot(A3(half), bf(jnp.concatenate([pre(blk(4)), ones], axis=0)))
                    users = [((half, 0), 1, [(v, 1) for v in quads(r[:, :h])]),
                             ((half, 1), 1, [(v, 1) for v in quads(r[:, h:])])]
                else:
                    i = int(c)
                    Bv = rhs_op(i, *[blk(k) if k in RHS_USES[i] else None for k in range(4)])
                    bq = quads(Bv)
                    sub = {}
                    very_last = mode == 'fine' and pos_ == len(order) - 1 and len(USERS[i]) == 1
                    sleft = {q: n - 1 for q, n in NTERMS.items()}
                    nb = even.get(pos_, 0)
                    rhs = {}
                    cuts = {1: [(0, 0, 48), (0, 48, 80), (0, 80, 112), (0, 112, Q)],
                            2: [(0, 0, 80), (0, 80, Q), (1, 0, 80), (1, 80, Q)],
                            3: [(0, 0, 112), (1, 0, 112), (2, 0, 112), (0, 112, Q), (1, 112, Q), (2, 112, Q)]}
                    for n_, kc in enumerate(subs[i]):
                        if n_ < 7 - nb:
                            v = rhs_op(int(kc), *bq)
                            mk = dot(Asub(i, int(kc)), bf(pre(v) if n_ == tsub[pos_] else v))
                        else:
                            if n_ == 7 - nb:
                                for n2 in range(n_, 7):
                                    v = rhs_op(int(subs[i][n2]), *bq)
                                    rhs[n2] = [bf(pre(v) if n2 == tsub[pos_] else v)]
                                for t, r0, r1 in cuts[nb]:
                                    rhs[n_ + t].append(dot(Asub(i, int(subs[i][n_ + t]))[r0:r1], rhs[n_ + t][0]))
                            mk = jnp.concatenate(rhs[n_][1:], axis=0)
                        for q, sg in USERS[int(kc)]:
                            accum(sub, q, mk, sg)
                            sleft[q] -= 1
                            if very_last and sleft[q] == 0:
                                (q0, sg0), = USERS[i]
                                accum(acc, (q0, q), sub[q][0], sub[q][1] * sg0)
                                o, so = acc[q0, q]
                                assert so > 0
                                region = (2 * s + q0[0], pl.ds(q[0] * Q, Q),
                                          pl.ds(c0 + q0[1] * h + q[1] * (h // 2), h // 2))
                                obuf[region] = bf(o)
                                write(region)
                    if very_last:
                        continue
                    r = [sub[sq] for sq in QUADS]
                    users = [(q, sg, r) for q, sg in USERS[i]]
                for q, sg, v in users:
                    for sq, (vq, sv) in zip(QUADS, v):
                        accum(acc, (q, sq), vq, sg * sv)
                    left[q] -= 1
                    if left[q] == 0:
                        assert all(acc[q, sq][1] > 0 for sq in QUADS)
                        o = jnp.concatenate([cat([acc[q, (0, 0)][0], acc[q, (0, 1)][0]]),
                                             cat([acc[q, (1, 0)][0], acc[q, (1, 1)][0]])], axis=0)
                        obuf[2 * s + q[0], :, c0 + q[1] * h:c0 + (q[1] + 1) * h] = bf(o)
                        if mode == 'fine':
                            write((2 * s + q[0], slice(None), pl.ds(c0 + q[1] * h, h)))
            return (cat([u[0] for u in done]), cat([u[1] for u in done])) if done else None

        head_rd[0].wait()
        t0 = [stats_tile(*k) for k in tiles_of((0, 0))]
        stat = cat([u[0] for u in t0]), cat([u[1] for u in t0])
        evens = [{} for _ in range(nhead)]
        npass, last_prod = 0, None
        for q in range(nhead + 1):
            for p_ in range(9):
                if (q, p_) in BARS or q == nhead:
                    if npass % 4:
                        evens[last_prod[0]][last_prod[1]] = npass % 4
                    npass = 0
                if q == nhead:
                    break
                if conf_of(('H', q))[0][p_] not in 'tb':
                    npass, last_prod = npass + 7, (q, p_)
        for q in range(nhead):
            waits = {p_: [head_rd[n + 1].wait] for n, (q_, p_) in enumerate(BARS) if q_ == q}
            if 0 in waits:
                waits.pop(0)[0]()
            stat = chunk(at(0, q), stat, tiles_of(at(0, q + 1)), conf_of(('H', q)), None, waits, evens[q])

        def put(stat):
            st_ref[0:8, 0:CN] = jnp.broadcast_to(stat[0], (8, CN))
            st_ref[8:16, 0:CN] = jnp.broadcast_to(stat[1], (8, CN))

        get = lambda: (st_ref[0:1, 0:CN], st_ref[8:9, 0:CN])
        put(stat)

        def body(i, carry):
            s0 = s_loop + i * SL
            rd_desc(s0 + 1, SL, 0, B, loop_sem0 + i).wait()
            wr_slabs(0, s_loop + IW * SL - 1, i == IW)
            stat = get()
            for j in range(NLOOP):
                stat = chunk(at(s0, j + 1), stat, tiles_of(at(s0, j + 2)), conf_of(('L', j)))
                if j % 4 == 0:
                    wr_slabs(s0 + j // 2 - 1, 2, i >= IW)
            while pend:
                pend.pop(0)()
            put(stat)
            return carry

        lax.fori_loop(0, NG, body, 0)

        post_rd.wait()
        stat = get()
        for j in range(NPOST):
            last = j + 1 == NPOST
            s, c0 = at(s_post, j + 1)
            stat = chunk((s, c0), stat, [] if last else tiles_of(at(s_post, j + 2)), conf_of(('P', j)),
                         'fine' if last else None, None, {8: (49 * NPOST) % 4} if last else {})
            if j == 0:
                wr_slabs(s - 1, 2)
            elif s + 1 < S and c0 > 0:
                wr_slabs(s, 1)
            elif s + 1 == S and not last:
                wr_slabs(s, 1, None, c0, CN, H)
        while pend:
            pend.pop(0)()
        pltpu.make_async_copy(obuf, o_hbm, wsem.at[0]).wait()

    @jax.jit
    def f(x, g, b, w):
        B, S, D = x.shape
        xt = jnp.transpose(x, (1, 2, 0))
        out = pl.pallas_call(
            kern,
            in_specs=[pl.BlockSpec(memory_space=pl.ANY)] * 4,
            out_specs=pl.BlockSpec(memory_space=pl.ANY),
            out_shape=jax.ShapeDtypeStruct((2 * S, D // 2, B), x.dtype),
            scratch_shapes=[
                pltpu.VMEM((S, D, B), BF16), pltpu.VMEM((2 * S, D // 2, B), BF16),
                pltpu.VMEM((D,), BF16), pltpu.VMEM((D,), BF16), pltpu.VMEM((D, D), BF16),
                pltpu.VMEM((D, 2 * KH), F32),
                pltpu.VMEM((D // 2 + 49 * (D // 8), 128), U32),
                pltpu.VMEM((16, 640), F32),
                pltpu.SemaphoreType.DMA((NSEM,)), pltpu.SemaphoreType.DMA((1,)),
            ],
            compiler_params=pltpu.CompilerParams(vmem_limit_bytes=110 * 1024 * 1024,
                                                 disable_bounds_checks=True, disable_semaphore_checks=True),
        )(xt, g, b, w)
        return jnp.transpose(out.reshape(S, D, B), (2, 0, 1))
    return f


_impl = build()


@jax.jit
def pallas_standalone__layernorm_linear__sampling_kernel(
    x: jax.Array,
    g: jax.Array,
    b: jax.Array,
    w: jax.Array,
):
    return _impl(x, g, b, w)
```
